```python
import jax
import jax.numpy as jnp

def _softmax(x, axis=-1):
    return jax.nn.softmax(x, axis=axis)
def _gelu(x):
    return jax.nn.gelu(x, approximate=True)
def _silu(x):
    return jax.nn.silu(x)
def _sigmoid(x):
    return jax.nn.sigmoid(x)
def _layernorm(x, axis=-1, eps=1e-5):
    m = jnp.mean(x, axis=axis, keepdims=True)
    v = jnp.var(x, axis=axis, keepdims=True)
    return (x - m) / jnp.sqrt(v + eps)
def _scatter_add(tgt, idx, src, axis=0):
    return tgt.at[idx].add(src)
def _segment_sum(src, seg, n):
    return jax.ops.segment_sum(src, seg, n)
class _Rng:
    def __init__(self, key):
        self._k = key
    def _next(self):
        self._k, sub = jax.random.split(self._k)
        return sub
    def normal(self, shape):
        return jax.random.normal(self._next(), shape, dtype=jnp.bfloat16)
    def randint(self, lo, hi, shape):
        return jax.random.randint(self._next(), shape, lo, hi, dtype=jnp.int32)
    def uniform(self, shape, lo=0.0, hi=1.0):
        return jax.random.uniform(self._next(), shape, jnp.bfloat16, lo, hi)
    def permutation(self, n):
        return jax.random.permutation(self._next(), n)


kernel_name = 'standalone__detection_seg_fpn_lateral__vision'

def setup_inputs():
    _rng = _Rng(jax.random.key(int.from_bytes(__import__("os").urandom(4), "little")))
    _w = (lambda a: (lambda t: t.astype(jnp.bfloat16) if jnp.issubdtype(t.dtype, jnp.floating) else t)(jnp.asarray(a)))
    H = W = (384 // 2) * 2
    C = 384
    k = 1
    return {
        "c_fine": _w((lambda *s: _rng.normal(s) * 0.05)(1, H, W, C)),
        "p_coarse": _w((lambda *s: _rng.normal(s) * 0.05)(1, H // 2, W // 2, C)),
        "w_lat": _w((lambda *s: _rng.normal(s) * 0.05)(C, C)),
        "w_out": _w((lambda *s: _rng.normal(s) * 0.05)(k, k, C, C)),
    }

def reference(c_fine, p_coarse, w_lat, w_out):
    B, H, W, C = c_fine.shape
    k = 1
    lat = jnp.einsum("bhwc,cd->bhwd", c_fine, w_lat)
    up = jnp.repeat(jnp.repeat(p_coarse, 2, axis=1), 2, axis=2)
    m = lat + up
    pad = k // 2
    mp = jnp.pad(m, ((0, 0), (pad, pad), (pad, pad), (0, 0)))
    o = None
    for di in range(k):
        for dj in range(k):
            t = jnp.einsum("bhwc,cd->bhwd", mp[:, di:di + H, dj:dj + W, :], w_out[di, dj])
            o = t if o is None else o + t
    return o
```

```python
import functools
import contextlib
import jax, jax.numpy as jnp
from jax import lax
import jax.experimental.pallas as pl
import jax.experimental.pallas.tpu as pltpu
f32 = jnp.float32; bf16 = jnp.bfloat16; u32 = jnp.uint32

def dot(a, b):
    return jnp.dot(a, b, preferred_element_type=f32)

def make(P=16, a=7, rows=48, G0=2, tail=(8, 4, 2, 1, 1), tailrows=48, scopes=False, wearly=2, rearly=768, vmem=120):
    sc = (lambda n: jax.named_scope(n)) if scopes else (lambda n: contextlib.nullcontext())
    def fn(c_fine, p_coarse, w_lat, w_out):
        B, H, W, C = c_fine.shape
        W2 = W // 2
        U = B * H // 2
        R = 2 * W
        n = U // P
        assert n * P == U and sum(tail) == P
        c4 = c_fine.reshape(U, R, C)
        p4 = p_coarse.reshape(U, W2, C)
        wo = w_out.reshape(C, C)
        nr = R // rows
        n0 = P // G0
        nt = len(tail)
        nmid = 2 * (n - 2)

        def kern(c_hbm, p_hbm, wl_hbm, wo_hbm, o_hbm, cbuf, pbuf, obuf, wl_ref, wo_ref, wf_ref, rs, ps, ws, s0c, s0p, wsem, tsem, rs2, ws2):
            def rd_main(k, slot):
                if rearly == 0:
                    return [pltpu.make_async_copy(p_hbm.at[pl.ds(k*P, P)], pbuf.at[slot], ps.at[slot]),
                            pltpu.make_async_copy(c_hbm.at[pl.ds(k*P, P)], cbuf.at[slot], rs.at[slot])]
                return [pltpu.make_async_copy(p_hbm.at[pl.ds(k*P, P)], pbuf.at[slot], ps.at[slot]),
                        pltpu.make_async_copy(c_hbm.at[pl.ds(k*P, P-1)], cbuf.at[slot, pl.ds(0, P-1)], rs.at[slot])] + (
                       [pltpu.make_async_copy(c_hbm.at[k*P + P-1, pl.ds(0, R - rearly)], cbuf.at[slot, P-1, pl.ds(0, R - rearly)], rs.at[slot])] if rearly < R else [])
            def rd_last(k, slot):
                if rearly == 0:
                    return []
                return [pltpu.make_async_copy(c_hbm.at[k*P + P-1, pl.ds(R - rearly, rearly)], cbuf.at[slot, P-1, pl.ds(R - rearly, rearly)], rs2.at[slot])]
            def rd0(g):
                return (pltpu.make_async_copy(p_hbm.at[pl.ds(g*G0, G0)], pbuf.at[0, pl.ds(g*G0, G0)], s0p.at[g]),
                        pltpu.make_async_copy(c_hbm.at[pl.ds(g*G0, G0)], cbuf.at[0, pl.ds(g*G0, G0)], s0c.at[g]))
            def wr1(k, slot, i, sem):
                return pltpu.make_async_copy(obuf.at[slot, :, pl.ds(i*rows, rows), :],
                                              o_hbm.at[pl.ds(k*P, P), pl.ds(i*rows, rows), :], sem.at[slot])
            def wr_main(k, slot):
                return [wr1(k, slot, i, ws) for i in range(nr - wearly)]
            def wr_last(k, slot):
                return [wr1(k, slot, i, ws2) for i in range(nr - wearly, nr)]
            def wr_tail(t):
                j0 = sum(tail[:t]); s = tail[t]; slot = (n - 1) % 2
                rr = tailrows if s > 1 else R
                return [pltpu.make_async_copy(obuf.at[slot, pl.ds(j0, s), pl.ds(i*rr, rr), :],
                                              o_hbm.at[pl.ds((n-1)*P + j0, s), pl.ds(i*rr, rr), :], tsem.at[t]) for i in range(R // rr)]
            def start_ordered(main, last):
                if not last:
                    for c in main: c.start()
                    return
                def f(i, _):
                    @pl.when(i == 0)
                    def _():
                        for c in main: c.start()
                    @pl.when(i == 1)
                    def _():
                        for c in last: c.start()
                lax.fori_loop(0, 2, f, None)

            cw = (pltpu.make_async_copy(wl_hbm, wl_ref, wsem.at[0]), pltpu.make_async_copy(wo_hbm, wo_ref, wsem.at[1]))
            for c in cw: c.start()
            def st0(g, _):
                for c in rd0(g): c.start()
            lax.fori_loop(0, n0, st0, None)
            start_ordered(rd_main(1, 1), rd_last(1, 1))
            with sc("w_wt"):
                for c in cw: c.wait()
            wf_ref[...] = dot(wl_ref[...], wo_ref[...]).astype(bf16)

            def compute(u, _):
                slot = (u // P) % 2; j = u % P
                q = dot(pbuf[slot, j], wo_ref[...])
                for r in (0, W):
                    x = pltpu.bitcast(cbuf[slot, j, pl.ds(r, W), :], u32)
                    xe = pltpu.unpack_elementwise(x, index=0, packed_dtype=bf16, unpacked_dtype=f32).astype(bf16)
                    xo = pltpu.unpack_elementwise(x, index=1, packed_dtype=bf16, unpacked_dtype=f32).astype(bf16)
                    y = dot(jnp.concatenate([xe, xo], axis=0), wf_ref[...])
                    o = pltpu.pack_elementwise([y[:W2] + q, y[W2:] + q], packed_dtype=bf16)
                    obuf[slot, j, pl.ds(r, W), :] = pltpu.bitcast(o, bf16)

            def seg(s, u0):
                m = s - n0
                k = 1 + m // 2; slot = k % 2
                @pl.when(s < n0)
                def _():
                    with sc("w_r0"):
                        for c in rd0(s): c.wait()
                @pl.when((m >= 0) & (m <= nmid) & (m % 2 == 0))
                def _():
                    with sc("w_r"):
                        for c in rd_main(k, slot): c.wait()
                    start_ordered(wr_main(k - 1, 1 - slot), wr_last(k - 1, 1 - slot))
                    for c in rd_last(k, slot): c.wait()
                @pl.when((m >= 0) & (m < nmid) & (m % 2 == 1))
                def _():
                    with sc("w_w"):
                        for c in wr_main(k - 1, 1 - slot): c.wait()
                    start_ordered(rd_main(k + 1, 1 - slot), rd_last(k + 1, 1 - slot))
                    for c in wr_last(k - 1, 1 - slot): c.wait()
                cnt = jnp.where(s < n0, G0, jnp.where(m % 2 == 0, a, P - a))
                for t in range(nt):
                    cnt = jnp.where(m == nmid + t, tail[t], cnt)
                lax.fori_loop(u0, u0 + cnt, compute, None)
                for t in range(nt):
                    @pl.when(m == nmid + t)
                    def _():
                        for c in wr_tail(t): c.start()
                return u0 + cnt
            lax.fori_loop(0, n0 + nmid + nt, seg, 0)
            with sc("w_tail"):
                for c in wr_main(n - 2, (n - 2) % 2) + wr_last(n - 2, (n - 2) % 2): c.wait()
            with sc("w_tail2"):
                for t in range(nt):
                    for c in wr_tail(t): c.wait()

        out = pl.pallas_call(
            kern,
            in_specs=[pl.BlockSpec(memory_space=pl.ANY)] * 4,
            out_specs=pl.BlockSpec(memory_space=pl.ANY),
            out_shape=jax.ShapeDtypeStruct((U, R, C), c_fine.dtype),
            scratch_shapes=[pltpu.VMEM((2, P, R, C), bf16), pltpu.VMEM((2, P, W2, C), bf16), pltpu.VMEM((2, P, R, C), bf16),
                            pltpu.VMEM((C, C), bf16), pltpu.VMEM((C, C), bf16), pltpu.VMEM((C, C), bf16),
                            pltpu.SemaphoreType.DMA((2,)), pltpu.SemaphoreType.DMA((2,)), pltpu.SemaphoreType.DMA((2,)),
                            pltpu.SemaphoreType.DMA((n0,)), pltpu.SemaphoreType.DMA((n0,)), pltpu.SemaphoreType.DMA((2,)),
                            pltpu.SemaphoreType.DMA((nt,)), pltpu.SemaphoreType.DMA((2,)), pltpu.SemaphoreType.DMA((2,))],
            compiler_params=pltpu.CompilerParams(vmem_limit_bytes=vmem*1024*1024),
        )(c4, p4, w_lat, wo)
        return out.reshape(B, H, W, C)
    return fn


@jax.jit
def pallas_standalone__detection_seg_fpn_lateral__vision_kernel(c_fine, p_coarse, w_lat, w_out):
    return make()(c_fine, p_coarse, w_lat, w_out)
```

```python
import jax
import jax.numpy as jnp
from jax import lax
import jax.experimental.pallas as pl
import jax.experimental.pallas.tpu as pltpu

GROUP = 6
STEP = 2
IN_SLOTS = 12
OUT_SLOTS = 16
READ_PIECES = 8
WRITE_PIECES = 16
NCOL = 6


def _schedule(n_groups, phases=(24, 42, 68), lead=11):
    spg = GROUP // STEP
    n_steps = n_groups * spg
    w1_start, r2_start, w2_start = (n_steps * x // 96 for x in phases)
    r1 = n_groups // 2
    w1 = n_groups * 3 // 8
    rows = []
    for i in range(n_steps):
        need = i // spg + 1
        done = i // spg
        if i < w1_start:
            reads, read_fence = min(5 * r1, lead + 3 * i), 0
            writes, write_fence = 0, 0
        elif i < r2_start:
            reads, read_fence = 5 * r1, r1
            writes, write_fence = min(w1, done, 4 + 2 * (i - w1_start) // 3), 0
        elif i < w2_start:
            reads, read_fence = min(5 * n_groups, 5 * r1 + 5 + 3 * (i - r2_start)), r1
            writes, write_fence = w1, w1
        else:
            reads, read_fence = 5 * n_groups, n_groups
            writes, write_fence = min(done, w1 + 4 + 2 * (i - w2_start) // 3), w1
        rows.append((max(write_fence, need - OUT_SLOTS), reads // 5 * 4 + min(reads % 5, 4),
                     reads // 5, max(read_fence, need), writes, need))

    prev = (0, 4, 1, 0, 0, 0)
    for i, row in enumerate(rows):
        assert all(a >= b for a, b in zip(row, prev))
        assert row[0] <= prev[4]
        assert max(-(-row[1] // 4), row[2]) - IN_SLOTS <= i // spg
        assert 4 * row[3] <= row[1] and row[5] <= row[2]
        assert row[4] <= i // spg
        assert min(row[3], row[5]) > i // spg
        assert i // spg + 1 - OUT_SLOTS <= row[0]
        prev = row
    assert prev[1:4] == (4 * n_groups, n_groups, n_groups) and prev[5] == n_groups
    return rows


def _dot(a, b):
    return jnp.dot(a, b, preferred_element_type=jnp.float32)


def _fpn_lateral(c_fine, p_coarse, w_lat, w_out, schedule=_schedule, interpret=False):
    B, H, W, C = c_fine.shape
    W2 = W // 2
    units = B * H // 2
    n_groups = units // GROUP
    assert w_out.shape == (1, 1, C, C) and p_coarse.shape == (B, H // 2, W2, C)
    assert n_groups * GROUP == units and C % 128 == 0
    half = GROUP // 2
    rd_rows = W2 // READ_PIECES
    wr_rows = 2 * W // WRITE_PIECES
    assert rd_rows % 8 == 0 and wr_rows % 8 == 0
    table = schedule(n_groups)
    dtype = c_fine.dtype

    def kernel(c_hbm, p_hbm, wl_hbm, wo_hbm, o_hbm,
               cbuf, pbuf, obuf, wl_ref, wo_ref, wf_ref, up_ref, tab_ref,
               c_sem, p_sem, o_sem, w_sem):
        def group(g):
            return pl.ds(g * GROUP, GROUP)

        def start_slice(src, dst, sem, g, row0):
            s = lax.rem(g, IN_SLOTS)
            for i in range(READ_PIECES):
                rows = pl.ds(row0 + i * rd_rows, rd_rows)
                for b in range(2):
                    pltpu.make_async_copy(
                        src.at[pl.ds(g * GROUP + b * half, half), rows, :],
                        dst.at[pl.ds(s * GROUP + b * half, half), rows, :],
                        sem.at[s]).start(priority=b)

        def start_c(j, _):
            start_slice(c_hbm, cbuf, c_sem, lax.div(j, 4), pl.multiple_of(lax.rem(j, 4) * W2, W2))

        def start_p(g, _):
            start_slice(p_hbm, pbuf, p_sem, g, 0)

        def start_o(g, _):
            s = lax.rem(g, OUT_SLOTS)
            for i in range(WRITE_PIECES):
                rows = pl.ds(i * wr_rows, wr_rows)
                pltpu.make_async_copy(
                    obuf.at[group(s), rows, :], o_hbm.at[group(g), rows, :], o_sem.at[s]).start()

        def wait_c(g, _):
            s = lax.rem(g, IN_SLOTS)
            pltpu.make_async_copy(c_hbm.at[group(g)], cbuf.at[group(s)], c_sem.at[s]).wait()

        def wait_p(g, _):
            s = lax.rem(g, IN_SLOTS)
            pltpu.make_async_copy(p_hbm.at[group(g)], pbuf.at[group(s)], p_sem.at[s]).wait()

        def wait_o(g, _):
            s = lax.rem(g, OUT_SLOTS)
            pltpu.make_async_copy(obuf.at[group(s)], o_hbm.at[group(g)], o_sem.at[s]).wait()

        def compute(i):
            ui = lax.rem(i * STEP, IN_SLOTS * GROUP)
            uo = lax.rem(i * STEP, OUT_SLOTS * GROUP)
            for t in range(STEP):
                q = _dot(pbuf[ui + t], wo_ref[...])
                for k in range(C // 128):
                    for r in range(2):
                        up_ref[t, k, pl.ds(r, W2, stride=2), :] = q[:, k * 128:(k + 1) * 128]
                up = jnp.concatenate([up_ref[t, k] for k in range(C // 128)], axis=1)
                for r in (0, W):
                    y = _dot(cbuf[ui + t, pl.ds(r, W), :], wf_ref[...])
                    obuf[uo + t, pl.ds(r, W), :] = (y + up).astype(dtype)

        weights = (pltpu.make_async_copy(wl_hbm, wl_ref, w_sem.at[0]),
                   pltpu.make_async_copy(wo_hbm, wo_ref, w_sem.at[1]))
        for cp in weights:
            cp.start()
        lax.fori_loop(0, 4, start_c, None)
        start_p(jnp.int32(0), None)
        for i, row in enumerate(table):
            for j, v in enumerate(row):
                tab_ref[i * NCOL + j] = jnp.int32(v)
        for cp in weights:
            cp.wait()
        wf_ref[...] = _dot(wl_ref[...], wo_ref[...]).astype(dtype)

        def step(i, prev):
            cur = tuple(tab_ref[i * NCOL + j] for j in range(NCOL))
            for lo, hi, event in zip(prev, cur, (wait_o, start_c, start_p, wait_c, start_o, wait_p)):
                lax.fori_loop(lo, hi, event, None)
            compute(i)
            return cur

        lax.fori_loop(0, len(table), step, tuple(jnp.int32(v) for v in (0, 4, 1, 0, 0, 0)))
        lax.fori_loop(table[-1][4], n_groups, start_o, None)
        lax.fori_loop(table[-1][0], n_groups, wait_o, None)

    out = pl.pallas_call(
        kernel,
        in_specs=[pl.BlockSpec(memory_space=pl.ANY)] * 4,
        out_specs=pl.BlockSpec(memory_space=pl.ANY),
        out_shape=jax.ShapeDtypeStruct((units, 2 * W, C), dtype),
        scratch_shapes=[
            pltpu.VMEM((IN_SLOTS * GROUP, 2 * W, C), dtype),
            pltpu.VMEM((IN_SLOTS * GROUP, W2, C), dtype),
            pltpu.VMEM((OUT_SLOTS * GROUP, 2 * W, C), dtype),
            pltpu.VMEM((C, C), dtype),
            pltpu.VMEM((C, C), dtype),
            pltpu.VMEM((C, C), dtype),
            pltpu.VMEM((STEP, C // 128, W, 128), jnp.float32),
            pltpu.SMEM((len(table) * NCOL,), jnp.int32),
            pltpu.SemaphoreType.DMA((IN_SLOTS,)),
            pltpu.SemaphoreType.DMA((IN_SLOTS,)),
            pltpu.SemaphoreType.DMA((OUT_SLOTS,)),
            pltpu.SemaphoreType.DMA((2,)),
        ],
        compiler_params=pltpu.CompilerParams(
            vmem_limit_bytes=120 * 1024 * 1024, disable_bounds_checks=True),
        interpret=interpret,
    )(c_fine.reshape(units, 2 * W, C), p_coarse.reshape(units, W2, C), w_lat, w_out.reshape(C, C))
    return out.reshape(B, H, W, C)


@jax.jit
def pallas_standalone__detection_seg_fpn_lateral__vision_kernel(
    c_fine: jax.Array,
    p_coarse: jax.Array,
    w_lat: jax.Array,
    w_out: jax.Array,
):
    return _fpn_lateral(c_fine, p_coarse, w_lat, w_out)
```
